```python
import os as _os
_os.environ.setdefault("JAX_PLATFORMS", "cpu")
import jax
import jax.numpy as jnp

def _softmax(x, axis=-1):
    return jax.nn.softmax(x, axis=axis)
def _gelu(x):
    return jax.nn.gelu(x, approximate=True)
def _silu(x):
    return jax.nn.silu(x)
def _sigmoid(x):
    return jax.nn.sigmoid(x)
def _layernorm(x, axis=-1, eps=1e-5):
    m = jnp.mean(x, axis=axis, keepdims=True)
    v = jnp.var(x, axis=axis, keepdims=True)
    return (x - m) / jnp.sqrt(v + eps)
def _scatter_add(tgt, idx, src, axis=0):
    return tgt.at[idx].add(src)
def _segment_sum(src, seg, n):
    return jax.ops.segment_sum(src, seg, n)
class _Rng:
    def __init__(self, key):
        self._k = key
    def _next(self):
        self._k, sub = jax.random.split(self._k)
        return sub
    def normal(self, shape):
        return jax.random.normal(self._next(), shape, dtype=jnp.bfloat16)
    def randint(self, lo, hi, shape):
        return jax.random.randint(self._next(), shape, lo, hi, dtype=jnp.int32)
    def uniform(self, shape, lo=0.0, hi=1.0):
        return jax.random.uniform(self._next(), shape, jnp.bfloat16, lo, hi)
    def permutation(self, n):
        return jax.random.permutation(self._next(), n)


kernel_name = 'standalone__gqa_softmax__near_ridge'

def setup_inputs():
    _rng = _Rng(jax.random.key(int.from_bytes(__import__("os").urandom(4), "little")))
    _w = (lambda a: (lambda t: t.astype(jnp.bfloat16) if jnp.issubdtype(t.dtype, jnp.floating) else t)(jnp.asarray(a)))
    B, Hq, Hkv, Sq, Sk, D = 8, 16, 8, 160, 2048, 256
    return {
        "q": _w((lambda *s: _rng.normal(s) * 0.05)(B, Hq, Sq, D)),
        "k": _w((lambda *s: _rng.normal(s) * 3.2)(B, Hkv, Sk, D)),
        "v": _w((lambda *s: _rng.normal(s) * 0.05)(B, Hkv, Sk, D)),
    }

def reference(q, k, v):
    B, Hq, Sq, D = q.shape
    Hkv = k.shape[1]
    rep = Hq // Hkv
    k = jnp.repeat(k, rep, axis=1)
    v = jnp.repeat(v, rep, axis=1)
    scale = D ** -0.5
    scores = jnp.einsum("bhqd,bhkd->bhqk", q, k) * scale
    p = _softmax(scores, axis=-1)
    return jnp.einsum("bhqk,bhkd->bhqd", p, v)
```

```python
import math
import jax
import jax.numpy as jnp
import jax.experimental.pallas as pl
import jax.experimental.pallas.tpu as pltpu


def make(N1=15, G1=3, G2=6, CH=256, NOBC=True, PVCH=256, ORDER=0, ONEP=True):
    nb = 6
    @jax.jit
    def pallas_standalone__gqa_softmax__near_ridge_kernel(q, k, v):
        B, Hq, Sq, D = q.shape
        _, Hkv, Sk, _ = k.shape
        rep = Hq // Hkv
        M = rep * Sq
        NH = B * Hkv
        NC = Sk // CH
        NS = NH - 1
        assert N1 % G1 == 0 and (NS - N1) % G2 == 0 and G2 % 2 == 0
        c2 = (D ** -0.5) * math.log2(math.e)
        q2 = q.reshape(NH, M, D)
        k2 = k.reshape(NH, Sk, D)
        v2 = v.reshape(NH, Sk, D)
        KO, VO, QO = 0, Sk, 2 * Sk

        def kernel(q_hbm, k_hbm, v_hbm, o_hbm, buf, obuf, s_c, s_a, s_b, mx_c, l_c, o_c, p_a, p_b,
                   sem, sem_q0, sem_o, rsem):
            def k_copy(h, slot):
                return pltpu.make_async_copy(k_hbm.at[h], buf.at[slot, pl.ds(KO, Sk)], sem.at[slot])
            def v_copy(h, slot):
                return pltpu.make_async_copy(v_hbm.at[h], buf.at[slot, pl.ds(VO, Sk)], sem.at[slot])
            def q_copy(h, slot, s=None):
                return pltpu.make_async_copy(q_hbm.at[h], buf.at[slot, pl.ds(QO, M)],
                                             sem.at[slot] if s is None else s)
            def wait_all(slot):
                pltpu.make_async_copy(buf.at[slot], buf.at[slot], sem.at[slot]).wait()
            def o_copy(h):
                return pltpu.make_async_copy(obuf.at[h], o_hbm.at[h], sem_o)
            def issue(x, slot):
                @pl.when(x + 1 < NH)
                def _():
                    k_copy(x + 1, slot).start()
                    q_copy(x + 1, slot).start()
                @pl.when(x < NH)
                def _():
                    v_copy(x, slot).start()
            def order_barrier():
                pl.semaphore_signal(rsem, 1)
                pl.semaphore_wait(rsem, 1)

            def A(slot, c, sdst, mx):
                s = jax.lax.dot_general(buf[slot, QO:QO + M, :],
                                        buf[slot, KO + c * CH:KO + (c + 1) * CH, :],
                                        (((1,), (1,)), ((), ())),
                                        preferred_element_type=jnp.float32)
                sdst[:, c * CH:(c + 1) * CH] = s
                t = s[:, :128]
                for j in range(1, CH // 128):
                    t = jnp.maximum(t, s[:, j * 128:(j + 1) * 128])
                return t if mx is None else jnp.maximum(mx, t)

            def E(c, ssrc, pdst, m, l):
                s = ssrc[:, c * CH:(c + 1) * CH]
                p = jnp.exp2((s - m) * c2)
                pdst[:, c * CH:(c + 1) * CH] = p.astype(jnp.bfloat16)
                t = p[:, :128]
                for j in range(1, CH // 128):
                    t = t + p[:, j * 128:(j + 1) * 128]
                return t if l is None else l + t

            def PV(slot, c, psrc, o):
                d = jnp.dot(psrc[:, c * PVCH:(c + 1) * PVCH], buf[slot, VO + c * PVCH:VO + (c + 1) * PVCH, :],
                            preferred_element_type=jnp.float32)
                return d if o is None else o + d

            def finish(h, l, o):
                lsum = jnp.sum(l, axis=-1, keepdims=True)
                obuf[h] = (o / lsum).astype(obuf.dtype)

            sl0 = nb - 1
            k_copy(0, sl0).start()
            q_copy(0, sl0, sem_q0).start()
            for x in range(4):
                order_barrier()
                k_copy(x + 1, x).start()
                q_copy(x + 1, x).start()
                v_copy(x, x).start()
            l_c[...] = jnp.ones(l_c.shape, l_c.dtype)
            o_c[...] = jnp.zeros(o_c.shape, o_c.dtype)
            k_copy(0, sl0).wait()
            q_copy(0, sl0, sem_q0).wait()
            mx = None
            for c in range(NC):
                mx = A(sl0, c, s_c, mx)
            mx_c[...] = mx

            def group(t0, G, W, slot_of):
                sbufs = [s_c] + [(s_a, s_b)[j % 2] for j in range(G - 1)] + [s_c]
                for j in range(G):
                    t = t0 + j
                    sl = slot_of(j)
                    if j % W == 0:
                        for w in range(W):
                            wait_all(slot_of(j + w))
                        for w in range(W):
                            issue(t + 4 + w, slot_of(j + 4 + w))
                    if j == 0:
                        mx = mx_c[...]; l = l_c[...]; o = o_c[...]
                    m = jnp.max(mx, axis=-1, keepdims=True)
                    hp = jnp.maximum(t - 1, 0)
                    finish(hp, l, o)

                    @pl.when(t >= 1)
                    def _():
                        o_copy(hp).start()

                    mx = None; l = None; o = None
                    pb = p_a if ONEP else (p_a, p_b)[j % 2]
                    if ORDER == 0:
                        for c in range(NC):
                            mx = A(sl, c, sbufs[j + 1], mx)
                            l = E(c, sbufs[j], pb, m, l)
                        for c in range(Sk // PVCH):
                            o = PV(sl, c, pb, o)
                    else:
                        for c in range(NC):
                            mx = A(sl, c, sbufs[j + 1], mx)
                            l = E(c, sbufs[j], pb, m, l)
                            o = PV(sl, c, pb, o)
                mx_c[...] = mx; l_c[...] = l; o_c[...] = o

            def body1(g, carry):
                t0 = g * G1
                if G1 % nb == 0:
                    group(t0, G1, 1, lambda j: j % nb)
                else:
                    group(t0, G1, 1, lambda j: jax.lax.rem(t0 + j, nb))
                return carry
            jax.lax.fori_loop(0, N1 // G1, body1, 0)

            def body2(g, carry):
                t0 = N1 + g * G2
                if G2 % nb == 0:
                    group(t0, G2, 2, lambda j: (N1 + j) % nb)
                else:
                    group(t0, G2, 2, lambda j: jax.lax.rem(t0 + j, nb))
                return carry
            jax.lax.fori_loop(0, (NS - N1) // G2, body2, 0)

            hl = NH - 1
            sl = hl % nb
            v_copy(hl, sl).wait()
            m = jnp.max(mx_c[...], axis=-1, keepdims=True)
            finish(hl - 1, l_c[...], o_c[...])
            o_copy(hl - 1).start()
            l = None; o = None
            for c in range(NC):
                l = E(c, s_c, p_a, m, l)
            for c in range(Sk // PVCH):
                o = PV(sl, c, p_a, o)
            finish(hl, l, o)
            o_copy(hl).start()
            pltpu.make_async_copy(obuf, obuf, sem_o).wait()

        out = pl.pallas_call(
            kernel,
            in_specs=[pl.BlockSpec(memory_space=pl.ANY)] * 3,
            out_specs=pl.BlockSpec(memory_space=pl.ANY),
            out_shape=jax.ShapeDtypeStruct((NH, M, D), q.dtype),
            scratch_shapes=[
                pltpu.VMEM((nb, 2 * Sk + M, D), k.dtype),
                pltpu.VMEM((NH, M, D), q.dtype),
                pltpu.VMEM((M, Sk), jnp.float32),
                pltpu.VMEM((M, Sk), jnp.float32),
                pltpu.VMEM((M, Sk), jnp.float32),
                pltpu.VMEM((M, 128), jnp.float32),
                pltpu.VMEM((M, 128), jnp.float32),
                pltpu.VMEM((M, D), jnp.float32),
                pltpu.VMEM((M, Sk), jnp.bfloat16),
                pltpu.VMEM((M, Sk), jnp.bfloat16),
                pltpu.SemaphoreType.DMA((nb,)),
                pltpu.SemaphoreType.DMA(()),
                pltpu.SemaphoreType.DMA(()),
                pltpu.SemaphoreType.REGULAR(()),
            ],
            compiler_params=pltpu.CompilerParams(
                vmem_limit_bytes=100 * 1024 * 1024,
                disable_bounds_checks=NOBC,
            ),
        )(q2, k2, v2)
        return out.reshape(B, Hq, Sq, D)
    return pallas_standalone__gqa_softmax__near_ridge_kernel


pallas_standalone__gqa_softmax__near_ridge_kernel = make(63, 3, 6, ONEP=False)
```

```python
import math

import jax
import jax.numpy as jnp
import jax.experimental.pallas as pl
import jax.experimental.pallas.tpu as pltpu

_CH = 256
_G = 2
_NB = 6
_PD = 4


@jax.jit
def pallas_standalone__gqa_softmax__near_ridge_kernel(
    q: jax.Array,
    k: jax.Array,
    v: jax.Array,
):
    B, Hq, Sq, D = q.shape
    _, Hkv, Sk, _ = k.shape
    rep = Hq // Hkv
    M = rep * Sq
    NH = B * Hkv
    CH, G, nb, PD = _CH, _G, _NB, _PD
    NC = Sk // CH
    NL = CH // 128
    NS = NH - 2
    assert Sk % CH == 0 and NS % G == 0 and G == 2 and PD < nb and NH > nb
    c2 = (D ** -0.5) * math.log2(math.e)
    KO, VO, QO = 0, Sk, 2 * Sk

    q2 = q.reshape(NH, M, D)
    k2 = k.reshape(NH, Sk, D)
    v2 = v.reshape(NH, Sk, D)

    def kernel(q_hbm, k_hbm, v_hbm, o_hbm, buf, obuf, s_c, s_a, mx_c, l_c, o_c,
               p_a, p_b, sem, sem_x, sem_o, rsem):
        def k_copy(h, slot, s=None):
            return pltpu.make_async_copy(
                k_hbm.at[h], buf.at[slot, pl.ds(KO, Sk)],
                sem.at[slot] if s is None else s)

        def q_copy(h, slot, s=None):
            return pltpu.make_async_copy(
                q_hbm.at[h], buf.at[slot, pl.ds(QO, M)],
                sem.at[slot] if s is None else s)

        def v_copy(h, slot):
            return pltpu.make_async_copy(
                v_hbm.at[h], buf.at[slot, pl.ds(VO, Sk)], sem.at[slot])

        def wait_slot(slot):
            pltpu.make_async_copy(buf.at[slot], buf.at[slot], sem.at[slot]).wait()

        def o_copy(h):
            return pltpu.make_async_copy(obuf.at[h], o_hbm.at[h], sem_o)

        def issue(x, slot):
            @pl.when(x + 1 < NH)
            def _():
                k_copy(x + 1, slot).start()
                q_copy(x + 1, slot).start()

            @pl.when(x < NH)
            def _():
                v_copy(x, slot).start()

        def order_barrier():
            pl.semaphore_signal(rsem, 1)
            pl.semaphore_wait(rsem, 1)

        def stage_a(slot, c, sdst, mx):
            s = jax.lax.dot_general(
                buf[slot, QO:QO + M, :],
                buf[slot, KO + c * CH:KO + (c + 1) * CH, :],
                (((1,), (1,)), ((), ())),
                preferred_element_type=jnp.float32)
            sdst[:, c * CH:(c + 1) * CH] = s
            t = s[:, :128]
            for j in range(1, NL):
                t = jnp.maximum(t, s[:, j * 128:(j + 1) * 128])
            return t if mx is None else jnp.maximum(mx, t)

        def stage_e(c, ssrc, pdst, mb, l):
            ps = []
            for j in range(NL):
                lo = c * CH + j * 128
                ps.append(jnp.exp2((ssrc[:, lo:lo + 128] - mb) * c2))
            pdst[:, c * CH:(c + 1) * CH] = (
                jnp.concatenate(ps, axis=1).astype(jnp.bfloat16))
            t = ps[0]
            for j in range(1, NL):
                t = t + ps[j]
            return t if l is None else l + t

        def stage_pv(slot, c, psrc, o):
            d = jnp.dot(psrc[:, c * CH:(c + 1) * CH],
                        buf[slot, VO + c * CH:VO + (c + 1) * CH, :],
                        preferred_element_type=jnp.float32)
            return d if o is None else o + d

        def rowmax_b(mx):
            return jnp.broadcast_to(jnp.max(mx, axis=-1, keepdims=True), (M, 128))

        def finish(h, l, o):
            lsum = jnp.sum(l, axis=-1, keepdims=True)
            r = pl.reciprocal(lsum, approx=True)
            r = r * (2.0 - lsum * r)
            r = r * (2.0 - lsum * r)
            obuf[h] = (o * r).astype(obuf.dtype)
            o_copy(h).start()

        sl0 = nb - 1
        k_copy(0, sl0).start()
        q_copy(0, sl0).start()
        order_barrier()
        k_copy(1, 0, sem_x).start()
        q_copy(1, 0, sem_x).start()
        order_barrier()
        v_copy(0, 0).start()
        for x in range(1, PD + 1):
            order_barrier()
            k_copy(x + 1, x).start()
            q_copy(x + 1, x).start()
            v_copy(x, x).start()

        k_copy(0, sl0).wait()
        q_copy(0, sl0).wait()
        mx0 = None
        for c in range(NC):
            mx0 = stage_a(sl0, c, s_a, mx0)

        k_copy(1, 0, sem_x).wait()
        q_copy(1, 0, sem_x).wait()
        mx = None
        for c in range(NC):
            mx = stage_a(0, c, s_c, mx)
        mx_c[...] = mx

        v_copy(0, 0).wait()
        mb = rowmax_b(mx0)
        l = None
        o = None
        for c in range(NC):
            l = stage_e(c, s_a, p_b, mb, l)
        for c in range(NC):
            o = stage_pv(0, c, p_b, o)
        l_c[...] = l
        o_c[...] = o

        sbufs = (s_c, s_a, s_c)

        def body(g, carry):
            t0 = 1 + g * G
            for j in range(G):
                t = t0 + j
                sl = jax.lax.rem(t, nb)
                sn = jax.lax.rem(t + PD, nb)
                wait_slot(sl)
                if j == 0:
                    mx = mx_c[...]
                    l = l_c[...]
                    o = o_c[...]
                mb = rowmax_b(mx)
                finish(t - 1, l, o)
                pb = (p_a, p_b)[j % 2]
                mx = None
                l = None
                o = None
                for c in range(NC):
                    mx = stage_a(sl, c, sbufs[j + 1], mx)
                    l = stage_e(c, sbufs[j], pb, mb, l)
                for c in range(NC):
                    o = stage_pv(sl, c, pb, o)
                issue(t + PD, sn)
            mx_c[...] = mx
            l_c[...] = l
            o_c[...] = o
            return carry

        jax.lax.fori_loop(0, NS // G, body, 0)

        hl = NH - 1
        sl = hl % nb
        v_copy(hl, sl).wait()
        mb = rowmax_b(mx_c[...])
        finish(hl - 1, l_c[...], o_c[...])
        l = None
        o = None
        for c in range(NC):
            l = stage_e(c, s_c, p_a, mb, l)
        for c in range(NC):
            o = stage_pv(sl, c, p_a, o)
        finish(hl, l, o)
        pltpu.make_async_copy(obuf, o_hbm, sem_o).wait()

    out = pl.pallas_call(
        kernel,
        in_specs=[pl.BlockSpec(memory_space=pl.ANY)] * 3,
        out_specs=pl.BlockSpec(memory_space=pl.ANY),
        out_shape=jax.ShapeDtypeStruct((NH, M, D), q.dtype),
        scratch_shapes=[
            pltpu.VMEM((nb, 2 * Sk + M, D), k.dtype),
            pltpu.VMEM((NH, M, D), q.dtype),
            pltpu.VMEM((M, Sk), jnp.float32),
            pltpu.VMEM((M, Sk), jnp.float32),
            pltpu.VMEM((M, 128), jnp.float32),
            pltpu.VMEM((M, 128), jnp.float32),
            pltpu.VMEM((M, D), jnp.float32),
            pltpu.VMEM((M, Sk), jnp.bfloat16),
            pltpu.VMEM((M, Sk), jnp.bfloat16),
            pltpu.SemaphoreType.DMA((nb,)),
            pltpu.SemaphoreType.DMA(()),
            pltpu.SemaphoreType.DMA(()),
            pltpu.SemaphoreType.REGULAR(()),
        ],
        compiler_params=pltpu.CompilerParams(
            vmem_limit_bytes=100 * 1024 * 1024,
            disable_bounds_checks=True,
        ),
    )(q2, k2, v2)
    return out.reshape(B, Hq, Sq, D)
```
